```python
import os as _os
_os.environ.setdefault("JAX_PLATFORMS", "cpu")
import jax
import jax.numpy as jnp

def _softmax(x, axis=-1):
    return jax.nn.softmax(x, axis=axis)
def _gelu(x):
    return jax.nn.gelu(x, approximate=True)
def _silu(x):
    return jax.nn.silu(x)
def _sigmoid(x):
    return jax.nn.sigmoid(x)
def _layernorm(x, axis=-1, eps=1e-5):
    m = jnp.mean(x, axis=axis, keepdims=True)
    v = jnp.var(x, axis=axis, keepdims=True)
    return (x - m) / jnp.sqrt(v + eps)
def _scatter_add(tgt, idx, src, axis=0):
    return tgt.at[idx].add(src)
def _segment_sum(src, seg, n):
    return jax.ops.segment_sum(src, seg, n)
class _Rng:
    def __init__(self, key):
        self._k = key
    def _next(self):
        self._k, sub = jax.random.split(self._k)
        return sub
    def normal(self, shape):
        return jax.random.normal(self._next(), shape, dtype=jnp.bfloat16)
    def randint(self, lo, hi, shape):
        return jax.random.randint(self._next(), shape, lo, hi, dtype=jnp.int32)
    def uniform(self, shape, lo=0.0, hi=1.0):
        return jax.random.uniform(self._next(), shape, jnp.bfloat16, lo, hi)
    def permutation(self, n):
        return jax.random.permutation(self._next(), n)


kernel_name = 'gated_mix__linear_attn_block__mixer_s_mlp__prompt'

def setup_inputs():
    _rng = _Rng(jax.random.key(int.from_bytes(__import__("os").urandom(4), "little")))
    _w = (lambda a: (lambda t: t.astype(jnp.bfloat16) if jnp.issubdtype(t.dtype, jnp.floating) else t)(jnp.asarray(a)))
    def _A_setup():
        B, S, D = 1, 2048, 640
        return {
            "x": _w((lambda *s: _rng.normal(s) * 0.05)(B, S, D)),
            "wqkv": _w((lambda *s: _rng.normal(s) * 0.8)(D, 3 * D)),
            "wo": _w((lambda *s: _rng.normal(s) * 0.1)(D, D)),
        }
    _A_in = _A_setup()

    def _B_setup():
        B, S, D, F = 1, 2048, 640, 1728
        return {
            "x":  _w((lambda *s: _rng.normal(s) * 0.05)(B, S, D)),
            "w1": _w((lambda *s: _rng.normal(s) * 0.2)(D, D) * (D ** -0.5)),
            "w2": _w((lambda *s: _rng.normal(s) * 0.2)(D, D) * (D ** -0.5)),
            "w3": _w((lambda *s: _rng.normal(s) * 0.2)(D, F) * (D ** -0.5)),
            "w4": _w((lambda *s: _rng.normal(s) * 0.2)(F, D) * (F ** -0.5)),
        }
    _B_in = _B_setup()

    return {
        "A_x": _A_in["x"],
        "A_wqkv": _A_in["wqkv"],
        "A_wo": _A_in["wo"],
        "B_x": _B_in["x"],
        "B_w1": _B_in["w1"],
        "B_w2": _B_in["w2"],
        "B_w3": _B_in["w3"],
        "B_w4": _B_in["w4"],
        "gate_w": _w((lambda *s: _rng.normal(s) * 0.05)(640) * 16.0),
    }

def reference(A_x, A_wqkv, A_wo, B_x, B_w1, B_w2, B_w3, B_w4, gate_w):
    def _A_ref(x, wqkv, wo):
        B, S, D = x.shape
        H = 32; Dh = D // H
        qkv = (lambda x, *d: x.transpose(*d))((x @ wqkv).reshape(B, S, 3, H, Dh), 2, 0, 3, 1, 4)
        q, k, v = qkv[0], qkv[1], qkv[2]
        phi = lambda t: jnp.where(t > 0, t + 1, jnp.exp(t)) + 1e-6
        pq, pk = phi(q), phi(k)
        kv = jnp.einsum("bhsd,bhse->bhde", pk, v)
        z = jnp.einsum("bhsd->bhd", pk)
        num = jnp.einsum("bhqd,bhde->bhqe", pq, kv)
        den = jnp.einsum("bhqd,bhd->bhq", pq, z)[..., None] + 1e-6
        o = num / den
        return (lambda x, *d: x.transpose(*d))(o, 0, 2, 1, 3).reshape(B, S, D) @ wo

    def _B_ref(x, w1, w2, w3, w4):
        B, S, D = x.shape
        h = _gelu(_layernorm(x, axis=-1) @ w1)
        c = D // 4
        g0 = jnp.pad(h[:, :, 0*c:1*c], ((0, 0), (1, 0), (0, 0)))[:, :S, :]
        g1 = jnp.pad(h[:, :, 1*c:2*c], ((0, 0), (0, 1), (0, 0)))[:, 1:, :]
        g2 = jnp.pad(h[:, :, 2*c:3*c], ((0, 0), (2, 0), (0, 0)))[:, :S, :]
        g3 = jnp.pad(h[:, :, 3*c:   ], ((0, 0), (0, 2), (0, 0)))[:, 2:, :]
        hs = jnp.concatenate([g0, g1, g2, g3], axis=-1) @ w2
        x1 = x + hs
        h2 = _gelu(_layernorm(x1, axis=-1) @ w3) @ w4
        return x1 + h2

    x = A_x
    g = _sigmoid((x * gate_w).sum(-1, keepdims=True))
    a = _A_ref(x, A_wqkv, A_wo)
    b = _B_ref(x, B_w1, B_w2, B_w3, B_w4)
    return g * a + (1 - g) * b
```

```python
import functools
import jax
import jax.numpy as jnp
from jax import lax
import jax.experimental.pallas as pl
import jax.experimental.pallas.tpu as pltpu

S = 2048
D = 640
F = 1728
H = 32
DH = 20
T1 = 256
T2 = 256
HALO = 8
BF = jnp.bfloat16
F32 = jnp.float32

_C1 = 0.7978845608028654
_C2 = 0.7978845608028654 * 0.044715


def _gelu(x):
    return 0.5 * x * (1.0 + jnp.tanh(x * (_C1 + _C2 * (x * x))))


def _phi(t):
    return jnp.where(t > 0, t + 1.0, jnp.exp(jnp.minimum(t, 0.0))) + 1e-6


def _ln(x):
    m = jnp.mean(x, axis=-1, keepdims=True)
    xc = x - m
    v = jnp.mean(xc * xc, axis=-1, keepdims=True)
    return xc * lax.rsqrt(v + 1e-5)


def _dot(a, b):
    return jnp.dot(a, b, preferred_element_type=F32)


def _dot_nt(a, b):
    return lax.dot_general(a, b, (((1,), (1,)), ((), ())), preferred_element_type=F32)


_WIN = [(0, 144), (112, 272), (240, 400), (368, 528), (496, 640)]


def _kernel(ax_hbm, wqkv_hbm, wo_hbm, w1_hbm, w2_hbm, w3_hbm, w4_hbm, gw_ref,
            out_hbm,
            ax, wqkv, wo, w1, w2, w3, w4,
            hbuf, pkt, wkt, wqtp, tmp, mp, zp, outv,
            sem_ax, sem_w, sem_out):
    n1 = S // T1
    n2 = S // T2

    def ax_copy(i):
        return pltpu.make_async_copy(ax_hbm.at[0, pl.ds(i * T1, T1), :],
                                     ax.at[pl.ds(i * T1, T1), :], sem_ax.at[i])

    def out_copy(i):
        return pltpu.make_async_copy(outv.at[pl.ds(i * T2, T2), :],
                                     out_hbm.at[0, pl.ds(i * T2, T2), :], sem_out.at[i])

    wk_copy = pltpu.make_async_copy(wqkv_hbm.at[:, pl.ds(D, D)], wqkv.at[:, pl.ds(D, D)], sem_w.at[0])
    w1_copy = pltpu.make_async_copy(w1_hbm, w1, sem_w.at[1])
    wq_copy = pltpu.make_async_copy(wqkv_hbm.at[:, pl.ds(0, D)], wqkv.at[:, pl.ds(0, D)], sem_w.at[2])
    wv_copy = pltpu.make_async_copy(wqkv_hbm.at[:, pl.ds(2 * D, D)], wqkv.at[:, pl.ds(2 * D, D)], sem_w.at[3])
    wo_copy = pltpu.make_async_copy(wo_hbm, wo, sem_w.at[4])
    w2_copy = pltpu.make_async_copy(w2_hbm, w2, sem_w.at[5])
    w3_copy = pltpu.make_async_copy(w3_hbm, w3, sem_w.at[6])
    w4_copy = pltpu.make_async_copy(w4_hbm, w4, sem_w.at[7])

    wk_copy.start()
    ax_copy(0).start()
    w1_copy.start()
    for i in range(1, n1):
        ax_copy(i).start()
    wq_copy.start()
    wv_copy.start()
    wo_copy.start()
    w2_copy.start()
    w3_copy.start()
    w4_copy.start()

    hbuf[pl.ds(0, HALO), :] = jnp.zeros((HALO, D), F32)
    hbuf[pl.ds(HALO + S, HALO), :] = jnp.zeros((HALO, D), F32)

    wk_copy.wait()
    wkt[...] = wqkv[:, D:2 * D].astype(F32).T.astype(BF)
    w1_copy.wait()

    def p1(i, zacc):
        r0 = pl.multiple_of(i * T1, T1)
        ax_copy(i).wait()
        xa = ax[pl.ds(r0, T1), :]
        kt = _dot_nt(wkt[...], xa)
        pk = _phi(kt)
        pkb = pk.astype(BF)
        pkt[:, pl.ds(r0, T1)] = pkb
        pkf = pkb.astype(F32)
        for c in range(T1 // 128):
            zacc = zacc + pkf[:, c * 128:(c + 1) * 128]
        xb = xa.astype(F32)
        h = _gelu(_dot(_ln(xb).astype(BF), w1[...]))
        hbuf[pl.ds(HALO + r0, T1), :] = h
        return zacc

    zacc = lax.fori_loop(0, n1, p1, jnp.zeros((D, 128), F32))

    wq_copy.wait()
    for c in range(5):
        tmp[c] = wqkv[128 * c:128 * (c + 1), 0:D].astype(F32).T
    for d in range(DH):
        for c in range(5):
            wqtp[d * H:(d + 1) * H, 128 * c:128 * (c + 1)] = tmp[c, pl.ds(d, H, stride=DH), :].astype(BF)

    P = _dot(pkt[...], ax[...]).astype(BF)
    wv_copy.wait()
    wo_copy.wait()
    for c in range(5):
        tmp[c] = jnp.zeros((D, 128), F32)
    tmp[5] = zacc
    for j, (a, b) in enumerate(_WIN):
        g = _dot(P[a:b, :], wqkv[:, 2 * D + 128 * j:2 * D + 128 * (j + 1)])
        rh = (lax.broadcasted_iota(jnp.int32, (b - a, 128), 0) + a) // DH
        ch = (lax.broadcasted_iota(jnp.int32, (b - a, 128), 1) + 128 * j) // DH
        g = jnp.where(rh == ch, g, 0.0).astype(BF)
        mj = _dot(g, wo[128 * j:128 * (j + 1), :])
        for c in range(5):
            tmp[c, a:b, :] += mj[:, 128 * c:128 * (c + 1)]
    for d in range(DH):
        for c in range(5):
            mp[d * H:(d + 1) * H, 128 * c:128 * (c + 1)] = tmp[c, pl.ds(d, H, stride=DH), :].astype(BF)
        zp[d * H:(d + 1) * H, :] = tmp[5, pl.ds(d, H, stride=DH), :]
    zrow = jnp.sum(zp[...].T, axis=0, keepdims=True)

    w2_copy.wait()
    w3_copy.wait()
    w4_copy.wait()
    gw = gw_ref[...].astype(F32).reshape(1, D)

    def p2(i, carry):
        r0 = pl.multiple_of(i * T2, T2)
        xa = ax[pl.ds(r0, T2), :]
        q = _dot_nt(xa, wqtp[...])
        pq = _phi(q)
        s = pq * zrow
        den = s[:, 0:128]
        for c in range(1, 5):
            den = den + s[:, c * 128:(c + 1) * 128]
        den = den + pltpu.roll(den, 32, 1)
        den = den + pltpu.roll(den, 64, 1)
        den = den + 1e-6
        g = jax.nn.sigmoid(jnp.sum(xa.astype(F32) * gw, axis=-1, keepdims=True))
        r = g / den
        pqn = jnp.concatenate([pq[:, c * 128:(c + 1) * 128] * r for c in range(5)], axis=1).astype(BF)
        a = _dot(pqn, mp[...])

        lane = lax.broadcasted_iota(jnp.int32, (T2, 128), 1)

        def hw(off, c):
            win = hbuf[pl.ds(r0, T2 + 2 * HALO), c * 128:(c + 1) * 128]
            return win[HALO + off:HALO + off + T2, :]
        t0 = hw(-1, 0)
        t1 = jnp.where(lane < 32, hw(-1, 1), hw(1, 1))
        t2 = jnp.where(lane < 64, hw(1, 2), hw(-2, 2))
        t3 = jnp.where(lane < 96, hw(-2, 3), hw(2, 3))
        t4 = hw(2, 4)
        hs = jnp.concatenate([t0, t1, t2, t3, t4], axis=1).astype(BF)
        x1 = xa.astype(F32) + _dot(hs, w2[...])
        hid = _gelu(_dot_nt(_ln(x1).astype(BF), w3[...])).astype(BF)
        b = x1 + _dot(hid, w4[...])
        outv[pl.ds(r0, T2), :] = (a + (1.0 - g) * b).astype(BF)
        out_copy(i).start()
        return carry

    lax.fori_loop(0, n2, p2, 0)
    for i in range(n2):
        out_copy(i).wait()


@jax.jit
def pallas_gated_mix__linear_attn_block__mixer_s_mlp__prompt_kernel(
    A_x, A_wqkv, A_wo, B_x, B_w1, B_w2, B_w3, B_w4, gate_w,
):
    any_spec = pl.BlockSpec(memory_space=pltpu.HBM)
    n1 = S // T1
    n2 = S // T2
    scratch = [
        pltpu.VMEM((S, D), BF),
        pltpu.VMEM((D, 3 * D), BF),
        pltpu.VMEM((D, D), BF),
        pltpu.VMEM((D, D), BF),
        pltpu.VMEM((D, D), BF),
        pltpu.VMEM((F, D), BF),
        pltpu.VMEM((F, D), BF),
        pltpu.VMEM((S + 2 * HALO, D), F32),
        pltpu.VMEM((D, S), BF),
        pltpu.VMEM((D, D), BF),
        pltpu.VMEM((D, D), BF),
        pltpu.VMEM((6, D, 128), F32),
        pltpu.VMEM((D, D), BF),
        pltpu.VMEM((D, 128), F32),
        pltpu.VMEM((S, D), BF),
        pltpu.SemaphoreType.DMA((n1,)),
        pltpu.SemaphoreType.DMA((8,)),
        pltpu.SemaphoreType.DMA((n2,)),
    ]
    return pl.pallas_call(
        _kernel,
        out_shape=jax.ShapeDtypeStruct((1, S, D), BF),
        in_specs=[any_spec] * 7 + [pl.BlockSpec(memory_space=pltpu.VMEM)],
        out_specs=any_spec,
        scratch_shapes=scratch,
        compiler_params=pltpu.CompilerParams(vmem_limit_bytes=100 * 1024 * 1024),
    )(A_x, A_wqkv, A_wo, B_w1, B_w2, B_w3.T, B_w4, gate_w)
```

```python
import jax
import jax.numpy as jnp
from jax import lax
import jax.experimental.pallas as pl
import jax.experimental.pallas.tpu as pltpu

S = 2048
D = 640
F = 1728
H = 32
FM = 1664
DH = 20
CX = 256
XSEG = [(0, 256), (256, 1024), (1024, 2048)]
TB = 512
MCH = [128] * 15 + [64, 64]
T2 = 512
HALO = 8
RB = 16
OSPLIT = [(0, 256), (256, 384), (384, 512)]
BF = jnp.bfloat16
F32 = jnp.float32

_C1 = 0.7978845608028654
_C2 = 0.7978845608028654 * 0.044715


def _gelu(x):
    return 0.5 * x * (1.0 + jnp.tanh(x * (_C1 + _C2 * (x * x))))


def _phi(t):
    return jnp.where(t > 0, t + 1.0, jnp.exp(jnp.minimum(t, 0.0))) + 1e-6


def _ln(x):
    m = jnp.mean(x, axis=-1, keepdims=True)
    xc = x - m
    v = jnp.mean(xc * xc, axis=-1, keepdims=True)
    return xc * lax.rsqrt(v + 1e-5)


def _dot(a, b):
    return jnp.dot(a, b, preferred_element_type=F32)


def _dot_nt(a, b):
    return lax.dot_general(a, b, (((1,), (1,)), ((), ())), preferred_element_type=F32)


_WIN = [(0, 144), (112, 272), (240, 400), (368, 528), (496, 640)]


def _kernel(ax_hbm, wqkv_hbm, wo_hbm, w1_hbm, w2_hbm, w3_hbm, w4_hbm, gw_hbm,
            out_hbm,
            ax, wq, wk, wv, wo, w1, w2, w3, w4, gwv,
            hbuf, wqtp, tmp, tq, mp, zp, pacc, zacc, x1s, lns, outv,
            sem_ax, sem_w, sem_out):
    n2 = S // T2

    def ax_copy(i):
        lo, hi = XSEG[i]
        return pltpu.make_async_copy(ax_hbm.at[0, pl.ds(lo, hi - lo), :],
                                     ax.at[pl.ds(lo, hi - lo), :], sem_ax.at[i])

    def out_copy(i, k):
        lo, hi = OSPLIT[k]
        return pltpu.make_async_copy(outv.at[pl.ds(i * T2 + lo, hi - lo), :],
                                     out_hbm.at[0, pl.ds(i * T2 + lo, hi - lo), :],
                                     sem_out.at[i * len(OSPLIT) + k])

    wk_copy = pltpu.make_async_copy(wqkv_hbm.at[:, pl.ds(D, D)], wk, sem_w.at[0])
    w1_copy = pltpu.make_async_copy(w1_hbm, w1, sem_w.at[1])
    wq_copy = pltpu.make_async_copy(wqkv_hbm.at[:, pl.ds(0, D)], wq, sem_w.at[2])
    wv_copy = pltpu.make_async_copy(wqkv_hbm.at[:, pl.ds(2 * D, D)], wv, sem_w.at[3])
    wo_copy = pltpu.make_async_copy(wo_hbm, wo, sem_w.at[4])
    w2_copy = pltpu.make_async_copy(w2_hbm, w2, sem_w.at[5])
    w3_copy = pltpu.make_async_copy(w3_hbm, w3, sem_w.at[6])
    w4_copy = pltpu.make_async_copy(w4_hbm, w4, sem_w.at[7])
    gw_copy = pltpu.make_async_copy(gw_hbm, gwv, sem_w.at[8])

    ax_copy(0).start()
    w1_copy.start()
    ax_copy(1).start()
    ax_copy(2).start()
    wk_copy.start()
    wq_copy.start()
    late = [w2_copy, wv_copy, wo_copy, gw_copy, w3_copy, w4_copy]

    for cc in range(5):
        hbuf[cc, pl.ds(0, HALO), :] = jnp.zeros((HALO, 128), F32)
        hbuf[cc, pl.ds(HALO + S, HALO), :] = jnp.zeros((HALO, 128), F32)
    pacc[...] = jnp.zeros((D, D), F32)
    zacc[...] = jnp.zeros((D, 128), F32)

    def h_store(r, h):
        for cc in range(5):
            hbuf[cc, HALO + r:HALO + r + h.shape[0], :] = h[:, 128 * cc:128 * (cc + 1)]

    def h_chunk(c, cs1):
        x = ax[c * CX:(c + 1) * CX, :]
        y = _dot(x, w1[...])
        for rb in range(0, CX, RB):
            xb = ax[c * CX + rb:c * CX + rb + RB, :].astype(F32)
            m = jnp.mean(xb, axis=-1, keepdims=True)
            xc = xb - m
            v = jnp.mean(xc * xc, axis=-1, keepdims=True)
            rstd = lax.rsqrt(v + 1e-5)
            h_store(c * CX + rb, _gelu((y[rb:rb + RB, :] - m * cs1) * rstd))

    def wq_t(cc):
        c0 = pl.multiple_of(cc * 128, 128)
        tq[...] = wq[pl.ds(c0, 128), :].astype(F32).T
        for d in range(DH):
            wqtp[d * H:(d + 1) * H, pl.ds(c0, 128)] = tq[pl.ds(d, H, stride=DH), :].astype(BF)

    ax_copy(0).wait()
    ln0 = jnp.concatenate(
        [_ln(ax[rb:rb + RB, :].astype(F32)).astype(BF) for rb in range(0, CX, RB)], axis=0)
    w1_copy.wait()
    h_store(0, _gelu(_dot(ln0, w1[...])))
    ax_copy(1).wait()
    cs1 = jnp.sum(w1[...].astype(F32), axis=0, keepdims=True)
    h_chunk(1, cs1)
    h_chunk(2, cs1)
    h_chunk(3, cs1)
    ax_copy(2).wait()
    h_chunk(4, cs1)
    h_chunk(5, cs1)
    h_chunk(6, cs1)
    h_chunk(7, cs1)
    wk_copy.wait()
    wq_copy.wait()

    def p1(i, carry):
        @pl.when(i == 1)
        def _():
            for cp in late:
                cp.start()
        r0 = pl.multiple_of(i * TB, TB)
        xa = ax[pl.ds(r0, TB), :]
        pkt = _phi(_dot(xa, wk[...])).T
        pkb = pkt.astype(BF)
        pkf = pkb.astype(F32)
        zs = pkf[:, 0:128]
        for c in range(1, TB // 128):
            zs = zs + pkf[:, c * 128:(c + 1) * 128]
        zacc[...] += zs
        pacc[...] += _dot(pkb, xa)
        if S // TB == 4:
            wq_t(i)
        return carry

    lax.fori_loop(0, S // TB, p1, 0)

    wv_copy.wait()
    wo_copy.wait()
    w2_copy.wait()

    def x1_chunk(r0, n):
        lane = lax.broadcasted_iota(jnp.int32, (n, 128), 1)

        def hw(off, cc):
            return hbuf[cc, pl.ds(r0 + HALO + off, n), :]
        t0 = hw(-1, 0)
        t1 = jnp.where(lane < 32, hw(-1, 1), hw(1, 1))
        t2 = jnp.where(lane < 64, hw(1, 2), hw(-2, 2))
        t3 = jnp.where(lane < 96, hw(-2, 3), hw(2, 3))
        t4 = hw(2, 4)
        hs = jnp.concatenate([t0, t1, t2, t3, t4], axis=1).astype(BF)
        x1 = ax[r0:r0 + n, :].astype(F32) + _dot(hs, w2[...])
        x1s[r0:r0 + n, :] = x1
        for rb in range(0, n, RB):
            lns[r0 + rb:r0 + rb + RB, :] = _ln(x1s[r0 + rb:r0 + rb + RB, :]).astype(BF)

    def g_step(j):
        a, b = _WIN[j]
        g = _dot(pacc[a:b, :].astype(BF), wv[:, 128 * j:128 * (j + 1)])
        rh = ((lax.broadcasted_iota(jnp.int32, (b - a, 1), 0) + a) * 3277) >> 16
        ch = ((lax.broadcasted_iota(jnp.int32, (1, 128), 1) + 128 * j) * 3277) >> 16
        g = jnp.where(rh == ch, g, 0.0).astype(BF)
        mj = _dot(g, wo[128 * j:128 * (j + 1), :])
        for c in range(5):
            tmp[c, a:b, :] += mj[:, 128 * c:128 * (c + 1)]

    for c in range(5):
        tmp[c] = jnp.zeros((D, 128), F32)
    tmp[5] = zacc[...]
    offs = [sum(MCH[:k]) for k in range(len(MCH))]
    x1_chunk(offs[0], MCH[0])
    g_step(0); g_step(1)
    x1_chunk(offs[1], MCH[1])
    g_step(2); g_step(3)
    x1_chunk(offs[2], MCH[2])
    g_step(4)
    for d in range(DH):
        zp[d * H:(d + 1) * H, :] = tmp[5, pl.ds(d, H, stride=DH), :]
    zrow = jnp.sum(zp[...].T, axis=0, keepdims=True)
    x1_chunk(offs[3], MCH[3])
    for d in range(DH):
        for c in range(5):
            mp[d * H:(d + 1) * H, 128 * c:128 * (c + 1)] = tmp[c, pl.ds(d, H, stride=DH), :].astype(BF)
    if S // TB == 4:
        wq_t(4)
    else:
        for cc in range(5):
            wq_t(cc)
    for k in range(4, len(MCH)):
        x1_chunk(offs[k], MCH[k])

    w3_copy.wait()
    w4_copy.wait()
    gw_copy.wait()
    gw = gwv[...].astype(F32).reshape(1, D)

    def p2(i, carry):
        r0 = pl.multiple_of(i * T2, T2)
        ln = lns[pl.ds(r0, T2), :]
        hid = _gelu(_dot_nt(ln, w3[0:FM, :])).astype(BF)
        hid_t = _gelu(_dot_nt(w3[FM:F, :], ln)).T.astype(BF)
        xa = ax[pl.ds(r0, T2), :]
        pq = _phi(_dot_nt(xa, wqtp[...]))
        s = pq * zrow
        den = s[:, 0:128]
        for c in range(1, 5):
            den = den + s[:, c * 128:(c + 1) * 128]
        den = den + pltpu.roll(den, 32, 1)
        den = den + pltpu.roll(den, 64, 1)
        den = den + 1e-6
        g = jax.nn.sigmoid(jnp.sum(xa.astype(F32) * gw, axis=-1, keepdims=True))
        r = g / den
        pqn = jnp.concatenate([pq[:, c * 128:(c + 1) * 128] * r for c in range(5)], axis=1).astype(BF)
        for k, (lo, hi) in enumerate(OSPLIT):
            a = _dot(pqn[lo:hi], mp[...])
            h2 = _dot(hid[lo:hi], w4[0:FM, :]) + _dot(hid_t[lo:hi], w4[FM:F, :])
            rr = pl.multiple_of(r0 + lo, 64)
            b = x1s[pl.ds(rr, hi - lo), :] + h2
            outv[pl.ds(rr, hi - lo), :] = (a + (1.0 - g[lo:hi]) * b).astype(BF)
            out_copy(i, k).start()
        return carry

    lax.fori_loop(0, n2, p2, 0)
    for i in range(n2):
        for k in range(len(OSPLIT)):
            out_copy(i, k).wait()


@jax.jit
def pallas_gated_mix__linear_attn_block__mixer_s_mlp__prompt_kernel(
    A_x, A_wqkv, A_wo, B_x, B_w1, B_w2, B_w3, B_w4, gate_w,
):
    hbm = pl.BlockSpec(memory_space=pltpu.HBM)
    nx = len(XSEG)
    n2 = S // T2
    scratch = [
        pltpu.VMEM((S, D), BF),
        pltpu.VMEM((D, D), BF),
        pltpu.VMEM((D, D), BF),
        pltpu.VMEM((D, D), BF),
        pltpu.VMEM((D, D), BF),
        pltpu.VMEM((D, D), BF),
        pltpu.VMEM((D, D), BF),
        pltpu.VMEM((F, D), BF),
        pltpu.VMEM((F, D), BF),
        pltpu.VMEM((D,), BF),
        pltpu.VMEM((5, S + 2 * HALO, 128), F32),
        pltpu.VMEM((D, D), BF),
        pltpu.VMEM((6, D, 128), F32),
        pltpu.VMEM((D, 128), F32),
        pltpu.VMEM((D, D), BF),
        pltpu.VMEM((D, 128), F32),
        pltpu.VMEM((D, D), F32),
        pltpu.VMEM((D, 128), F32),
        pltpu.VMEM((S, D), F32),
        pltpu.VMEM((S, D), BF),
        pltpu.VMEM((S, D), BF),
        pltpu.SemaphoreType.DMA((nx,)),
        pltpu.SemaphoreType.DMA((9,)),
        pltpu.SemaphoreType.DMA((n2 * len(OSPLIT),)),
    ]
    return pl.pallas_call(
        _kernel,
        out_shape=jax.ShapeDtypeStruct((1, S, D), BF),
        in_specs=[hbm] * 8,
        out_specs=hbm,
        scratch_shapes=scratch,
        compiler_params=pltpu.CompilerParams(vmem_limit_bytes=100 * 1024 * 1024),
    )(A_x, A_wqkv, A_wo, B_w1, B_w2, B_w3.T, B_w4, gate_w)
```

```python
import jax
import jax.numpy as jnp
from jax import lax
import jax.experimental.pallas as pl
import jax.experimental.pallas.tpu as pltpu

S = 2048
D = 640
F = 1728
FM = 1664
H = 32
DH = 20
CX = 256
XSEG = [(0, 256), (256, 768), (768, 2048)]
W1A = 256
TB = 512
MCH = [128] * 15 + [64, 64]
MORD = 'x g0 g1 x g2 g3 x g4 z x m0 m1 m2 m3 m4 q4'
T2 = 512
OSPLIT = [(0, 256), (256, 384), (384, 448), (448, 512)]
LNL = 128
HALO = 8
RB = 16
BF = jnp.bfloat16
F32 = jnp.float32

_C1 = 0.7978845608028654
_C2 = 0.7978845608028654 * 0.044715

_WIN = [(0, 144), (112, 272), (240, 400), (368, 528), (496, 640)]


def _gelu2(x):
    return x * (1.0 + jnp.tanh(x * (_C1 + _C2 * (x * x))))


def _gelu(x):
    return 0.5 * _gelu2(x)


def _phi(t):
    return jnp.where(t > 0, t + 1.0, jnp.exp(t)) + 1e-6


def _ln_stats(x):
    m = jnp.mean(x, axis=-1, keepdims=True)
    xc = x - m
    v = jnp.mean(xc * xc, axis=-1, keepdims=True)
    rstd = jnp.exp(-0.5 * jnp.log(v + 1e-5))
    return m, xc, rstd


def _ln(x):
    _, xc, rstd = _ln_stats(x)
    return xc * rstd


def _dot(a, b):
    return jnp.dot(a, b, preferred_element_type=F32)


def _dot_nt(a, b):
    return lax.dot_general(a, b, (((1,), (1,)), ((), ())), preferred_element_type=F32)


def _kernel(ax_hbm, wqkv_hbm, wo_hbm, w1_hbm, w2_hbm, w3_hbm, w4_hbm, gw_hbm,
            out_hbm,
            ax, wq, wk, wv, wo, w1, w2, w3, w4, gwv,
            hbuf, wqtp, tmp, tq, mp, zp, pacc, zacc, x1s, lns, outv,
            sem_ax, sem_w, sem_out):
    n2 = S // T2

    def ax_copy(i):
        lo, hi = XSEG[i]
        return pltpu.make_async_copy(ax_hbm.at[0, pl.ds(lo, hi - lo), :],
                                     ax.at[pl.ds(lo, hi - lo), :], sem_ax.at[i])

    def out_copy(i, k):
        lo, hi = OSPLIT[k]
        return pltpu.make_async_copy(outv.at[pl.ds(i * T2 + lo, hi - lo), :],
                                     out_hbm.at[0, pl.ds(i * T2 + lo, hi - lo), :],
                                     sem_out.at[i * len(OSPLIT) + k])

    wk_copy = pltpu.make_async_copy(wqkv_hbm.at[:, pl.ds(D, D)], wk, sem_w.at[0])
    w1a_copy = pltpu.make_async_copy(w1_hbm.at[:, pl.ds(0, W1A)], w1.at[:, pl.ds(0, W1A)], sem_w.at[1])
    w1b_copy = pltpu.make_async_copy(w1_hbm.at[:, pl.ds(W1A, D - W1A)], w1.at[:, pl.ds(W1A, D - W1A)],
                                     sem_w.at[9])
    wq_copy = pltpu.make_async_copy(wqkv_hbm.at[:, pl.ds(0, D)], wq, sem_w.at[2])
    wv_copy = pltpu.make_async_copy(wqkv_hbm.at[:, pl.ds(2 * D, D)], wv, sem_w.at[3])
    wo_copy = pltpu.make_async_copy(wo_hbm, wo, sem_w.at[4])
    w2_copy = pltpu.make_async_copy(w2_hbm, w2, sem_w.at[5])
    w3_copy = pltpu.make_async_copy(w3_hbm, w3, sem_w.at[6])
    w4_copy = pltpu.make_async_copy(w4_hbm, w4, sem_w.at[7])
    gw_copy = pltpu.make_async_copy(gw_hbm, gwv, sem_w.at[8])

    ax_copy(0).start()
    w1a_copy.start()
    w1b_copy.start()
    ax_copy(1).start()
    ax_copy(2).start()
    wk_copy.start()
    late = [w2_copy, wv_copy, wo_copy, gw_copy, w3_copy, w4_copy]

    for cc in range(5):
        hbuf[cc, pl.ds(0, HALO), :] = jnp.zeros((HALO, 128), F32)
        hbuf[cc, pl.ds(HALO + S, HALO), :] = jnp.zeros((HALO, 128), F32)
    pacc[...] = jnp.zeros((D, D), F32)
    zacc[...] = jnp.zeros((D, 128), F32)

    def h_chunk(c, cs1):
        y = _dot(ax[c * CX:(c + 1) * CX, :], w1[...])
        for rb in range(0, CX, RB):
            r = c * CX + rb
            m, _, rstd = _ln_stats(ax[r:r + RB, :].astype(F32))
            h = _gelu((y[rb:rb + RB, :] - m * cs1) * rstd)
            for cc in range(5):
                hbuf[cc, HALO + r:HALO + r + RB, :] = h[:, 128 * cc:128 * (cc + 1)]

    def wq_t(cc):
        c0 = cc * 128 if isinstance(cc, int) else pl.multiple_of(cc * 128, 128)
        tq[...] = wq[pl.ds(c0, 128), :].astype(F32).T
        for d in range(DH):
            wqtp[d * H:(d + 1) * H, pl.ds(c0, 128)] = tq[pl.ds(d, H, stride=DH), :].astype(BF)

    ax_copy(0).wait()
    ln0 = jnp.concatenate(
        [_ln(ax[rb:rb + RB, :].astype(F32)).astype(BF) for rb in range(0, CX, RB)]
        + [jnp.ones((16, D), BF)], axis=0)
    w1a_copy.wait()
    y0a = _dot(ln0, w1[:, 0:W1A])
    for cc in range(W1A // 128):
        hbuf[cc, HALO:HALO + CX, :] = _gelu(y0a[0:CX, 128 * cc:128 * (cc + 1)])
    w1b_copy.wait()
    y0b = _dot(ln0, w1[:, W1A:D])
    for cc in range(W1A // 128, 5):
        hbuf[cc, HALO:HALO + CX, :] = _gelu(y0b[0:CX, 128 * cc - W1A:128 * (cc + 1) - W1A])
    cs1 = jnp.concatenate([y0a[CX:CX + 1], y0b[CX:CX + 1]], axis=1)
    ax_copy(1).wait()
    wq_copy.start()
    for c in range(1, XSEG[1][1] // CX):
        h_chunk(c, cs1)
    ax_copy(2).wait()
    for c in range(XSEG[1][1] // CX, S // CX):
        h_chunk(c, cs1)
    wk_copy.wait()
    wq_copy.wait()

    def p1(i, carry):
        @pl.when(i == 1)
        def _():
            for cp in late:
                cp.start()
        r0 = pl.multiple_of(i * TB, TB)
        xa = ax[pl.ds(r0, TB), :]
        pkb = _phi(_dot(xa, wk[...])).T.astype(BF)
        pkf = pkb.astype(F32)
        zs = pkf[:, 0:128]
        for c in range(1, TB // 128):
            zs = zs + pkf[:, c * 128:(c + 1) * 128]
        zacc[...] += zs
        pacc[...] += _dot(pkb, xa)
        wq_t(i)
        return carry

    lax.fori_loop(0, S // TB, p1, 0)

    wv_copy.wait()
    wo_copy.wait()
    w2_copy.wait()

    def ln_rows(r0, n):
        for rb in range(0, n, RB):
            lns[r0 + rb:r0 + rb + RB, :] = _ln(x1s[r0 + rb:r0 + rb + RB, :]).astype(BF)

    def x1_chunk(r0, n):
        lane = lax.broadcasted_iota(jnp.int32, (n, 128), 1)

        def hw(off, cc):
            return hbuf[cc, pl.ds(r0 + HALO + off, n), :]
        t0 = hw(-1, 0)
        t1 = jnp.where(lane < 32, hw(-1, 1), hw(1, 1))
        t2 = jnp.where(lane < 64, hw(1, 2), hw(-2, 2))
        t3 = jnp.where(lane < 96, hw(-2, 3), hw(2, 3))
        t4 = hw(2, 4)
        hs = jnp.concatenate([t0, t1, t2, t3, t4], axis=1).astype(BF)
        x1s[r0:r0 + n, :] = ax[r0:r0 + n, :].astype(F32) + _dot(hs, w2[...])
        if r0 < S - LNL:
            ln_rows(r0, n)

    def g_step(j):
        a, b = _WIN[j]
        g = _dot(pacc[a:b, :].astype(BF), wv[:, 128 * j:128 * (j + 1)])
        rh = ((lax.broadcasted_iota(jnp.int32, (b - a, 1), 0) + a) * 3277) >> 16
        ch = ((lax.broadcasted_iota(jnp.int32, (1, 128), 1) + 128 * j) * 3277) >> 16
        g = jnp.where(rh == ch, g, 0.0).astype(BF)
        mj = _dot(g, wo[128 * j:128 * (j + 1), :])
        for c in range(5):
            tmp[c, a:b, :] += mj[:, 128 * c:128 * (c + 1)]

    def z_step():
        for d in range(DH):
            zp[d * H:(d + 1) * H, :] = tmp[5, pl.ds(d, H, stride=DH), :]
        return jnp.sum(zp[...].T, axis=0, keepdims=True)

    def m_perm(c):
        for d in range(DH):
            mp[d * H:(d + 1) * H, 128 * c:128 * (c + 1)] = tmp[c, pl.ds(d, H, stride=DH), :].astype(BF)

    for c in range(5):
        tmp[c] = jnp.zeros((D, 128), F32)
    tmp[5] = zacc[...]
    offs = [sum(MCH[:k]) for k in range(len(MCH))]
    k = 0
    for tok in MORD.split():
        if tok == 'x':
            x1_chunk(offs[k], MCH[k]); k += 1
        elif tok[0] == 'g':
            g_step(int(tok[1]))
        elif tok == 'z':
            zrow = z_step()
        elif tok[0] == 'm':
            m_perm(int(tok[1]))
        elif tok[0] == 'q':
            wq_t(int(tok[1]))
    while k < len(MCH):
        x1_chunk(offs[k], MCH[k]); k += 1

    w3_copy.wait()
    w4_copy.wait()
    gw_copy.wait()
    gw = gwv[...].astype(F32).reshape(1, D)

    def p2(i, carry):
        r0 = pl.multiple_of(i * T2, T2)
        ln = lns[pl.ds(r0, T2), :]
        hid = _gelu2(_dot_nt(ln, w3[0:FM, :])).astype(BF)
        hid_t = _gelu2(_dot_nt(w3[FM:F, :], ln)).T.astype(BF)
        xa = ax[pl.ds(r0, T2), :]
        pq = _phi(_dot_nt(xa, wqtp[...]))
        s = pq * zrow
        den = s[:, 0:128]
        for c in range(1, 5):
            den = den + s[:, c * 128:(c + 1) * 128]
        den = den + pltpu.roll(den, 32, 1)
        den = den + pltpu.roll(den, 64, 1)
        den = den + 1e-6
        g = jax.nn.sigmoid(jnp.sum(xa.astype(F32) * gw, axis=-1, keepdims=True))
        r = g / den
        pqn = jnp.concatenate([pq[:, c * 128:(c + 1) * 128] * r for c in range(5)], axis=1).astype(BF)
        for k, (lo, hi) in enumerate(OSPLIT):
            a = _dot(pqn[lo:hi], mp[...])
            h2 = _dot(hid[lo:hi], w4[0:FM, :]) + _dot(hid_t[lo:hi], w4[FM:F, :])
            rr = pl.multiple_of(r0 + lo, 64)
            b = x1s[pl.ds(rr, hi - lo), :] + 0.5 * h2
            outv[pl.ds(rr, hi - lo), :] = (a + (1.0 - g[lo:hi]) * b).astype(BF)
            out_copy(i, k).start()
        ln_rows(S - LNL, LNL)
        return carry

    lax.fori_loop(0, n2, p2, 0)
    for i in range(n2):
        for k in range(len(OSPLIT)):
            out_copy(i, k).wait()


@jax.jit
def pallas_gated_mix__linear_attn_block__mixer_s_mlp__prompt_kernel(
    A_x, A_wqkv, A_wo, B_x, B_w1, B_w2, B_w3, B_w4, gate_w,
):
    hbm = pl.BlockSpec(memory_space=pltpu.HBM)
    n2 = S // T2
    scratch = [
        pltpu.VMEM((S, D), BF),
        pltpu.VMEM((D, D), BF),
        pltpu.VMEM((D, D), BF),
        pltpu.VMEM((D, D), BF),
        pltpu.VMEM((D, D), BF),
        pltpu.VMEM((D, D), BF),
        pltpu.VMEM((D, D), BF),
        pltpu.VMEM((F, D), BF),
        pltpu.VMEM((F, D), BF),
        pltpu.VMEM((D,), BF),
        pltpu.VMEM((5, S + 2 * HALO, 128), F32),
        pltpu.VMEM((D, D), BF),
        pltpu.VMEM((6, D, 128), F32),
        pltpu.VMEM((D, 128), F32),
        pltpu.VMEM((D, D), BF),
        pltpu.VMEM((D, 128), F32),
        pltpu.VMEM((D, D), F32),
        pltpu.VMEM((D, 128), F32),
        pltpu.VMEM((S, D), F32),
        pltpu.VMEM((S, D), BF),
        pltpu.VMEM((S, D), BF),
        pltpu.SemaphoreType.DMA((len(XSEG),)),
        pltpu.SemaphoreType.DMA((10,)),
        pltpu.SemaphoreType.DMA((n2 * len(OSPLIT),)),
    ]
    return pl.pallas_call(
        _kernel,
        out_shape=jax.ShapeDtypeStruct((1, S, D), BF),
        in_specs=[hbm] * 8,
        out_specs=hbm,
        scratch_shapes=scratch,
        compiler_params=pltpu.CompilerParams(vmem_limit_bytes=100 * 1024 * 1024),
    )(A_x, A_wqkv, A_wo, B_w1, B_w2, B_w3.T, B_w4, gate_w)
```

```python
import jax
import jax.numpy as jnp
from jax import lax
import jax.experimental.pallas as pl
import jax.experimental.pallas.tpu as pltpu

S = 2048
D = 640
F = 1728
FM = 1664
H = 32
DH = 20
CX = 256
XSEG = [(0, 256), (256, 768), (768, 2048)]
HCH1 = [128] * 4
HCH2 = [128] * 10
W1A = 256
TB = 512
MCH = [128] * 15 + [64, 64]
MORD = 'x g0 g1 x g2 g3 x g4 z x m0 m1 m2 m3 m4 q4'
T2 = 512
OSPLIT = [(0, 256), (256, 384), (384, 448), (448, 512)]
LNL = 128
HALO = 8
RB = 16
BF = jnp.bfloat16
F32 = jnp.float32

_C1 = 0.7978845608028654
_C2 = 0.7978845608028654 * 0.044715

_WIN = [(0, 144), (112, 272), (240, 400), (368, 528), (496, 640)]


def _gelu2(x):
    return x * (1.0 + jnp.tanh(x * (_C1 + _C2 * (x * x))))


def _gelu(x):
    return 0.5 * _gelu2(x)


def _phi(t):
    return jnp.where(t > 0, t + 1.0, jnp.exp(t)) + 1e-6


def _ln_stats(x):
    m = jnp.mean(x, axis=-1, keepdims=True)
    xc = x - m
    v = jnp.mean(xc * xc, axis=-1, keepdims=True)
    rstd = jnp.exp(-0.5 * jnp.log(v + 1e-5))
    return m, xc, rstd


def _ln(x):
    _, xc, rstd = _ln_stats(x)
    return xc * rstd


def _dot(a, b):
    return jnp.dot(a, b, preferred_element_type=F32)


def _dot_nt(a, b):
    return lax.dot_general(a, b, (((1,), (1,)), ((), ())), preferred_element_type=F32)


def _kernel(ax_hbm, wqkv_hbm, wo_hbm, w1_hbm, w2_hbm, w3_hbm, w4_hbm, gw_hbm,
            out_hbm,
            ax, wq, wk, wv, wo, w1, w2, w3, w4, gwv,
            hbuf, wqtp, tmp, tq, mp, zp, pacc, zacc, x1s, lns, outv,
            sem_ax, sem_w, sem_out):
    n2 = S // T2

    def ax_copy(i):
        lo, hi = XSEG[i]
        return pltpu.make_async_copy(ax_hbm.at[0, pl.ds(lo, hi - lo), :],
                                     ax.at[pl.ds(lo, hi - lo), :], sem_ax.at[i])

    def out_copy(i, k):
        lo, hi = OSPLIT[k]
        return pltpu.make_async_copy(outv.at[pl.ds(i * T2 + lo, hi - lo), :],
                                     out_hbm.at[0, pl.ds(i * T2 + lo, hi - lo), :],
                                     sem_out.at[i * len(OSPLIT) + k])

    wk_copy = pltpu.make_async_copy(wqkv_hbm.at[:, pl.ds(D, D)], wk, sem_w.at[0])
    w1a_copy = pltpu.make_async_copy(w1_hbm.at[:, pl.ds(0, W1A)], w1.at[:, pl.ds(0, W1A)], sem_w.at[1])
    w1b_copy = pltpu.make_async_copy(w1_hbm.at[:, pl.ds(W1A, D - W1A)], w1.at[:, pl.ds(W1A, D - W1A)],
                                     sem_w.at[9])
    wq_copy = pltpu.make_async_copy(wqkv_hbm.at[:, pl.ds(0, D)], wq, sem_w.at[2])
    wv_copy = pltpu.make_async_copy(wqkv_hbm.at[:, pl.ds(2 * D, D)], wv, sem_w.at[3])
    wo_copy = pltpu.make_async_copy(wo_hbm, wo, sem_w.at[4])
    w2_copy = pltpu.make_async_copy(w2_hbm, w2, sem_w.at[5])
    w3_copy = pltpu.make_async_copy(w3_hbm, w3, sem_w.at[6])
    w4_copy = pltpu.make_async_copy(w4_hbm, w4, sem_w.at[7])
    gw_copy = pltpu.make_async_copy(gw_hbm, gwv, sem_w.at[8])

    ax_copy(0).start()
    w1a_copy.start()
    w1b_copy.start()
    ax_copy(1).start()
    ax_copy(2).start()
    wk_copy.start()
    late = [w2_copy, wv_copy, wo_copy, gw_copy, w3_copy, w4_copy]

    for cc in range(5):
        hbuf[cc, pl.ds(0, HALO), :] = jnp.zeros((HALO, 128), F32)
        hbuf[cc, pl.ds(HALO + S, HALO), :] = jnp.zeros((HALO, 128), F32)
    pacc[...] = jnp.zeros((D, D), F32)
    zacc[...] = jnp.zeros((D, 128), F32)

    def h_chunk(r0, n, cs1):
        y = _dot(ax[r0:r0 + n, :], w1[...])
        for rb in range(0, n, RB):
            r = r0 + rb
            m, _, rstd = _ln_stats(ax[r:r + RB, :].astype(F32))
            h = _gelu((y[rb:rb + RB, :] - m * cs1) * rstd)
            for cc in range(5):
                hbuf[cc, HALO + r:HALO + r + RB, :] = h[:, 128 * cc:128 * (cc + 1)]

    def wq_t(cc):
        c0 = cc * 128 if isinstance(cc, int) else pl.multiple_of(cc * 128, 128)
        tq[...] = wq[pl.ds(c0, 128), :].astype(F32).T
        for d in range(DH):
            wqtp[d * H:(d + 1) * H, pl.ds(c0, 128)] = tq[pl.ds(d, H, stride=DH), :].astype(BF)

    ax_copy(0).wait()
    ln0 = jnp.concatenate(
        [_ln(ax[rb:rb + RB, :].astype(F32)).astype(BF) for rb in range(0, CX, RB)]
        + [jnp.ones((16, D), BF)], axis=0)
    w1a_copy.wait()
    y0a = _dot(ln0, w1[:, 0:W1A])
    for cc in range(W1A // 128):
        hbuf[cc, HALO:HALO + CX, :] = _gelu(y0a[0:CX, 128 * cc:128 * (cc + 1)])
    w1b_copy.wait()
    y0b = _dot(ln0, w1[:, W1A:D])
    for cc in range(W1A // 128, 5):
        hbuf[cc, HALO:HALO + CX, :] = _gelu(y0b[0:CX, 128 * cc - W1A:128 * (cc + 1) - W1A])
    cs1 = jnp.concatenate([y0a[CX:CX + 1], y0b[CX:CX + 1]], axis=1)
    ax_copy(1).wait()
    wq_copy.start()
    r0 = XSEG[1][0]
    for n in HCH1:
        h_chunk(r0, n, cs1); r0 += n
    assert r0 == XSEG[1][1]
    ax_copy(2).wait()
    for n in HCH2:
        h_chunk(r0, n, cs1); r0 += n
    assert r0 == S
    wk_copy.wait()
    wq_copy.wait()

    def p1(i, carry):
        @pl.when(i == 1)
        def _():
            for cp in late:
                cp.start()
        r0 = pl.multiple_of(i * TB, TB)
        xa = ax[pl.ds(r0, TB), :]
        pkb = _phi(_dot(xa, wk[...])).T.astype(BF)
        pkf = pkb.astype(F32)
        zs = pkf[:, 0:128]
        for c in range(1, TB // 128):
            zs = zs + pkf[:, c * 128:(c + 1) * 128]
        zacc[...] += zs
        pacc[...] += _dot(pkb, xa)
        wq_t(i)
        return carry

    lax.fori_loop(0, S // TB, p1, 0)

    wv_copy.wait()
    wo_copy.wait()
    w2_copy.wait()

    def ln_rows(r0, n):
        for rb in range(0, n, RB):
            lns[r0 + rb:r0 + rb + RB, :] = _ln(x1s[r0 + rb:r0 + rb + RB, :]).astype(BF)

    def x1_chunk(r0, n):
        lane = lax.broadcasted_iota(jnp.int32, (n, 128), 1)

        def hw(off, cc):
            return hbuf[cc, pl.ds(r0 + HALO + off, n), :]
        t0 = hw(-1, 0)
        t1 = jnp.where(lane < 32, hw(-1, 1), hw(1, 1))
        t2 = jnp.where(lane < 64, hw(1, 2), hw(-2, 2))
        t3 = jnp.where(lane < 96, hw(-2, 3), hw(2, 3))
        t4 = hw(2, 4)
        hs = jnp.concatenate([t0, t1, t2, t3, t4], axis=1).astype(BF)
        x1s[r0:r0 + n, :] = ax[r0:r0 + n, :].astype(F32) + _dot(hs, w2[...])
        if r0 < S - LNL:
            ln_rows(r0, n)

    def g_step(j):
        a, b = _WIN[j]
        g = _dot(pacc[a:b, :].astype(BF), wv[:, 128 * j:128 * (j + 1)])
        rh = ((lax.broadcasted_iota(jnp.int32, (b - a, 1), 0) + a) * 3277) >> 16
        ch = ((lax.broadcasted_iota(jnp.int32, (1, 128), 1) + 128 * j) * 3277) >> 16
        g = jnp.where(rh == ch, g, 0.0).astype(BF)
        mj = _dot(g, wo[128 * j:128 * (j + 1), :])
        for c in range(5):
            tmp[c, a:b, :] += mj[:, 128 * c:128 * (c + 1)]

    def z_step():
        for d in range(DH):
            zp[d * H:(d + 1) * H, :] = tmp[5, pl.ds(d, H, stride=DH), :]
        return jnp.sum(zp[...].T, axis=0, keepdims=True)

    def m_perm(c):
        for d in range(DH):
            mp[d * H:(d + 1) * H, 128 * c:128 * (c + 1)] = tmp[c, pl.ds(d, H, stride=DH), :].astype(BF)

    for c in range(5):
        tmp[c] = jnp.zeros((D, 128), F32)
    tmp[5] = zacc[...]
    offs = [sum(MCH[:k]) for k in range(len(MCH))]
    k = 0
    for tok in MORD.split():
        if tok == 'x':
            x1_chunk(offs[k], MCH[k]); k += 1
        elif tok[0] == 'g':
            g_step(int(tok[1]))
        elif tok == 'z':
            zrow = z_step()
        elif tok[0] == 'm':
            m_perm(int(tok[1]))
        elif tok[0] == 'q':
            wq_t(int(tok[1]))
    while k < len(MCH):
        x1_chunk(offs[k], MCH[k]); k += 1

    w3_copy.wait()
    w4_copy.wait()
    gw_copy.wait()
    gw = gwv[...].astype(F32).reshape(1, D)

    def p2(i, carry):
        r0 = pl.multiple_of(i * T2, T2)
        ln = lns[pl.ds(r0, T2), :]
        hid = _gelu2(_dot_nt(ln, w3[0:FM, :])).astype(BF)
        hid_t = _gelu2(_dot_nt(w3[FM:F, :], ln)).T.astype(BF)
        xa = ax[pl.ds(r0, T2), :]
        pq = _phi(_dot_nt(xa, wqtp[...]))
        s = pq * zrow
        den = s[:, 0:128]
        for c in range(1, 5):
            den = den + s[:, c * 128:(c + 1) * 128]
        den = den + pltpu.roll(den, 32, 1)
        den = den + pltpu.roll(den, 64, 1)
        den = den + 1e-6
        g = jax.nn.sigmoid(jnp.sum(xa.astype(F32) * gw, axis=-1, keepdims=True))
        r = g / den
        pqn = jnp.concatenate([pq[:, c * 128:(c + 1) * 128] * r for c in range(5)], axis=1).astype(BF)
        for k, (lo, hi) in enumerate(OSPLIT):
            a = _dot(pqn[lo:hi], mp[...])
            h2 = _dot(hid[lo:hi], w4[0:FM, :]) + _dot(hid_t[lo:hi], w4[FM:F, :])
            rr = pl.multiple_of(r0 + lo, 64)
            b = x1s[pl.ds(rr, hi - lo), :] + 0.5 * h2
            outv[pl.ds(rr, hi - lo), :] = (a + (1.0 - g[lo:hi]) * b).astype(BF)
            out_copy(i, k).start()
        ln_rows(S - LNL, LNL)
        return carry

    lax.fori_loop(0, n2, p2, 0)
    for i in range(n2):
        for k in range(len(OSPLIT)):
            out_copy(i, k).wait()


@jax.jit
def pallas_gated_mix__linear_attn_block__mixer_s_mlp__prompt_kernel(
    A_x, A_wqkv, A_wo, B_x, B_w1, B_w2, B_w3, B_w4, gate_w,
):
    hbm = pl.BlockSpec(memory_space=pltpu.HBM)
    n2 = S // T2
    scratch = [
        pltpu.VMEM((S, D), BF),
        pltpu.VMEM((D, D), BF),
        pltpu.VMEM((D, D), BF),
        pltpu.VMEM((D, D), BF),
        pltpu.VMEM((D, D), BF),
        pltpu.VMEM((D, D), BF),
        pltpu.VMEM((D, D), BF),
        pltpu.VMEM((F, D), BF),
        pltpu.VMEM((F, D), BF),
        pltpu.VMEM((D,), BF),
        pltpu.VMEM((5, S + 2 * HALO, 128), F32),
        pltpu.VMEM((D, D), BF),
        pltpu.VMEM((6, D, 128), F32),
        pltpu.VMEM((D, 128), F32),
        pltpu.VMEM((D, D), BF),
        pltpu.VMEM((D, 128), F32),
        pltpu.VMEM((D, D), F32),
        pltpu.VMEM((D, 128), F32),
        pltpu.VMEM((S, D), F32),
        pltpu.VMEM((S, D), BF),
        pltpu.VMEM((S, D), BF),
        pltpu.SemaphoreType.DMA((len(XSEG),)),
        pltpu.SemaphoreType.DMA((10,)),
        pltpu.SemaphoreType.DMA((n2 * len(OSPLIT),)),
    ]
    return pl.pallas_call(
        _kernel,
        out_shape=jax.ShapeDtypeStruct((1, S, D), BF),
        in_specs=[hbm] * 8,
        out_specs=hbm,
        scratch_shapes=scratch,
        compiler_params=pltpu.CompilerParams(vmem_limit_bytes=100 * 1024 * 1024),
    )(A_x, A_wqkv, A_wo, B_w1, B_w2, B_w3.T, B_w4, gate_w)
```

```python
import jax
import jax.numpy as jnp
from jax import lax
import jax.experimental.pallas as pl
import jax.experimental.pallas.tpu as pltpu

S = 2048
D = 640
F = 1728
FM = 1664
H = 32
DH = 20
CX = 256
XSEG = [(0, 256), (256, 768), (768, 2048)]
HCH1 = [128] * 4
HCH2 = [128] * 10
W1A = 256
TB = 512
MCH = [128] * 15 + [64, 64]
MORD = 'x x a0 a1 a2 a3 a4 x x b0 b1 b2 b3 b4 z x x m0 m1 m2 m3 m4 q4'
T2 = 512
OSPLIT = [(0, 256), (256, 384), (384, 448), (448, 512)]
LNL = 64
HALO = 8
RB = 16
BF = jnp.bfloat16
F32 = jnp.float32

_C1 = 0.7978845608028654
_C2 = 0.7978845608028654 * 0.044715

_WIN = [(0, 144), (112, 272), (240, 400), (368, 528), (496, 640)]


def _gelu2(x):
    return x * (1.0 + jnp.tanh(x * (_C1 + _C2 * (x * x))))


def _gelu(x):
    return 0.5 * _gelu2(x)


def _phi(t):
    return jnp.where(t > 0, t + 1.0, jnp.exp(t)) + 1e-6


def _ln_stats(x):
    m = jnp.mean(x, axis=-1, keepdims=True)
    xc = x - m
    v = jnp.mean(xc * xc, axis=-1, keepdims=True)
    rstd = jnp.exp(-0.5 * jnp.log(v + 1e-5))
    return m, xc, rstd


def _ln(x):
    _, xc, rstd = _ln_stats(x)
    return xc * rstd


def _dot(a, b):
    return jnp.dot(a, b, preferred_element_type=F32)


def _dot_nt(a, b):
    return lax.dot_general(a, b, (((1,), (1,)), ((), ())), preferred_element_type=F32)


def _kernel(ax_hbm, wqkv_hbm, wo_hbm, w1_hbm, w2_hbm, w3_hbm, w4_hbm, gw_hbm,
            out_hbm,
            ax, wq, wk, wv, wo, w1, w2, w3, w4, gwv,
            hbuf, wqtp, tmp, tq, mp, zp, pacc, zacc, x1s, lns, outv,
            sem_ax, sem_w, sem_out):
    n2 = S // T2

    def ax_copy(i):
        lo, hi = XSEG[i]
        return pltpu.make_async_copy(ax_hbm.at[0, pl.ds(lo, hi - lo), :],
                                     ax.at[pl.ds(lo, hi - lo), :], sem_ax.at[i])

    def out_copy(i, k):
        lo, hi = OSPLIT[k]
        return pltpu.make_async_copy(outv.at[pl.ds(i * T2 + lo, hi - lo), :],
                                     out_hbm.at[0, pl.ds(i * T2 + lo, hi - lo), :],
                                     sem_out.at[i * len(OSPLIT) + k])

    wk_copy = pltpu.make_async_copy(wqkv_hbm.at[:, pl.ds(D, D)], wk, sem_w.at[0])
    w1a_copy = pltpu.make_async_copy(w1_hbm.at[:, pl.ds(0, W1A)], w1.at[:, pl.ds(0, W1A)], sem_w.at[1])
    w1b_copy = pltpu.make_async_copy(w1_hbm.at[:, pl.ds(W1A, D - W1A)], w1.at[:, pl.ds(W1A, D - W1A)],
                                     sem_w.at[9])
    wq_copy = pltpu.make_async_copy(wqkv_hbm.at[:, pl.ds(0, D)], wq, sem_w.at[2])
    wv_copy = pltpu.make_async_copy(wqkv_hbm.at[:, pl.ds(2 * D, D)], wv, sem_w.at[3])
    wo_copy = pltpu.make_async_copy(wo_hbm, wo, sem_w.at[4])
    w2_copy = pltpu.make_async_copy(w2_hbm, w2, sem_w.at[5])
    w3_copy = pltpu.make_async_copy(w3_hbm, w3, sem_w.at[6])
    w4_copy = pltpu.make_async_copy(w4_hbm, w4, sem_w.at[7])
    gw_copy = pltpu.make_async_copy(gw_hbm, gwv, sem_w.at[8])

    ax_copy(0).start()
    w1a_copy.start()
    w1b_copy.start()
    ax_copy(1).start()
    ax_copy(2).start()
    wk_copy.start()
    late = [w2_copy, wv_copy, wo_copy, gw_copy, w3_copy, w4_copy]

    for cc in range(5):
        hbuf[cc, pl.ds(0, HALO), :] = jnp.zeros((HALO, 128), F32)
        hbuf[cc, pl.ds(HALO + S, HALO), :] = jnp.zeros((HALO, 128), F32)
    pacc[...] = jnp.zeros((D, D), F32)
    zacc[...] = jnp.zeros((D, 128), F32)

    def h_chunk(r0, n, cs1):
        y = _dot(ax[r0:r0 + n, :], w1[...])
        for rb in range(0, n, RB):
            r = r0 + rb
            m, _, rstd = _ln_stats(ax[r:r + RB, :].astype(F32))
            h = _gelu((y[rb:rb + RB, :] - m * cs1) * rstd)
            for cc in range(5):
                hbuf[cc, HALO + r:HALO + r + RB, :] = h[:, 128 * cc:128 * (cc + 1)]

    def wq_t(cc):
        c0 = cc * 128 if isinstance(cc, int) else pl.multiple_of(cc * 128, 128)
        tq[...] = wq[pl.ds(c0, 128), :].astype(F32).T
        for d in range(DH):
            wqtp[d * H:(d + 1) * H, pl.ds(c0, 128)] = tq[pl.ds(d, H, stride=DH), :].astype(BF)

    ax_copy(0).wait()
    ln0 = jnp.concatenate(
        [_ln(ax[rb:rb + RB, :].astype(F32)).astype(BF) for rb in range(0, CX, RB)]
        + [jnp.ones((16, D), BF)], axis=0)
    w1a_copy.wait()
    y0a = _dot(ln0, w1[:, 0:W1A])
    for cc in range(W1A // 128):
        hbuf[cc, HALO:HALO + CX, :] = _gelu(y0a[0:CX, 128 * cc:128 * (cc + 1)])
    w1b_copy.wait()
    y0b = _dot(ln0, w1[:, W1A:D])
    for cc in range(W1A // 128, 5):
        hbuf[cc, HALO:HALO + CX, :] = _gelu(y0b[0:CX, 128 * cc - W1A:128 * (cc + 1) - W1A])
    cs1 = jnp.concatenate([y0a[CX:CX + 1], y0b[CX:CX + 1]], axis=1)
    ax_copy(1).wait()
    wq_copy.start()
    r0 = XSEG[1][0]
    for n in HCH1:
        h_chunk(r0, n, cs1); r0 += n
    assert r0 == XSEG[1][1]
    ax_copy(2).wait()
    for n in HCH2:
        h_chunk(r0, n, cs1); r0 += n
    assert r0 == S
    wk_copy.wait()
    wq_copy.wait()

    def p1(i, carry):
        @pl.when(i == 1)
        def _():
            for cp in late:
                cp.start()
        r0 = pl.multiple_of(i * TB, TB)
        xa = ax[pl.ds(r0, TB), :]
        pkb = _phi(_dot(xa, wk[...])).T.astype(BF)
        pkf = pkb.astype(F32)
        zs = pkf[:, 0:128]
        for c in range(1, TB // 128):
            zs = zs + pkf[:, c * 128:(c + 1) * 128]
        zacc[...] += zs
        pacc[...] += _dot(pkb, xa)
        wq_t(i)
        return carry

    lax.fori_loop(0, S // TB, p1, 0)

    wv_copy.wait()
    wo_copy.wait()
    w2_copy.wait()

    def ln_rows(r0, n):
        for rb in range(0, n, RB):
            lns[r0 + rb:r0 + rb + RB, :] = _ln(x1s[r0 + rb:r0 + rb + RB, :]).astype(BF)

    def x1_chunk(r0, n):
        lane = lax.broadcasted_iota(jnp.int32, (n, 128), 1)

        def hw(off, cc):
            return hbuf[cc, pl.ds(r0 + HALO + off, n), :]
        t0 = hw(-1, 0)
        t1 = jnp.where(lane < 32, hw(-1, 1), hw(1, 1))
        t2 = jnp.where(lane < 64, hw(1, 2), hw(-2, 2))
        t3 = jnp.where(lane < 96, hw(-2, 3), hw(2, 3))
        t4 = hw(2, 4)
        hs = jnp.concatenate([t0, t1, t2, t3, t4], axis=1).astype(BF)
        x1s[r0:r0 + n, :] = ax[r0:r0 + n, :].astype(F32) + _dot(hs, w2[...])
        if r0 < S - LNL:
            ln_rows(r0, n)

    gs = {}

    def g_a(j):
        a, b = _WIN[j]
        g = _dot(pacc[a:b, :].astype(BF), wv[:, 128 * j:128 * (j + 1)])
        rh = ((lax.broadcasted_iota(jnp.int32, (b - a, 1), 0) + a) * 3277) >> 16
        ch = ((lax.broadcasted_iota(jnp.int32, (1, 128), 1) + 128 * j) * 3277) >> 16
        gs[j] = jnp.where(rh == ch, g, 0.0).astype(BF)

    def g_b(j):
        a, b = _WIN[j]
        mj = _dot(gs[j], wo[128 * j:128 * (j + 1), :])
        for c in range(5):
            tmp[c, a:b, :] += mj[:, 128 * c:128 * (c + 1)]

    def g_step(j):
        g_a(j)
        g_b(j)

    def z_step():
        for d in range(DH):
            zp[d * H:(d + 1) * H, :] = tmp[5, pl.ds(d, H, stride=DH), :]
        return jnp.sum(zp[...].T, axis=0, keepdims=True)

    def m_perm(c):
        for d in range(DH):
            mp[d * H:(d + 1) * H, 128 * c:128 * (c + 1)] = tmp[c, pl.ds(d, H, stride=DH), :].astype(BF)

    for c in range(5):
        tmp[c] = jnp.zeros((D, 128), F32)
    tmp[5] = zacc[...]
    offs = [sum(MCH[:k]) for k in range(len(MCH))]
    k = 0
    for tok in MORD.split():
        if tok == 'x':
            x1_chunk(offs[k], MCH[k]); k += 1
        elif tok[0] == 'a':
            g_a(int(tok[1]))
        elif tok[0] == 'b':
            g_b(int(tok[1]))
        elif tok[0] == 'g':
            g_step(int(tok[1]))
        elif tok == 'z':
            zrow = z_step()
        elif tok[0] == 'm':
            m_perm(int(tok[1]))
        elif tok[0] == 'q':
            wq_t(int(tok[1]))
    while k < len(MCH):
        x1_chunk(offs[k], MCH[k]); k += 1

    w3_copy.wait()
    w4_copy.wait()
    gw_copy.wait()
    gw = gwv[...].astype(F32).reshape(1, D)

    def p2(i, carry):
        r0 = pl.multiple_of(i * T2, T2)
        xa = ax[pl.ds(r0, T2), :]
        pq = _phi(_dot_nt(xa, wqtp[...]))
        s = pq * zrow
        den = s[:, 0:128]
        for c in range(1, 5):
            den = den + s[:, c * 128:(c + 1) * 128]
        den = den + pltpu.roll(den, 32, 1)
        den = den + pltpu.roll(den, 64, 1)
        den = den + 1e-6
        g = jax.nn.sigmoid(jnp.sum(xa.astype(F32) * gw, axis=-1, keepdims=True))
        r = g / den
        pqn = jnp.concatenate([pq[:, c * 128:(c + 1) * 128] * r for c in range(5)], axis=1).astype(BF)
        ln = lns[pl.ds(r0, T2), :]
        hid = _gelu2(_dot_nt(ln, w3[0:FM, :])).astype(BF)
        hid_t = _gelu2(_dot_nt(w3[FM:F, :], ln)).T.astype(BF)
        for k, (lo, hi) in enumerate(OSPLIT):
            a = _dot(pqn[lo:hi], mp[...])
            h2 = _dot(hid[lo:hi], w4[0:FM, :]) + _dot(hid_t[lo:hi], w4[FM:F, :])
            rr = pl.multiple_of(r0 + lo, 64)
            b = x1s[pl.ds(rr, hi - lo), :] + 0.5 * h2
            outv[pl.ds(rr, hi - lo), :] = (a + (1.0 - g[lo:hi]) * b).astype(BF)
            out_copy(i, k).start()
        ln_rows(S - LNL, LNL)
        return carry

    lax.fori_loop(0, n2, p2, 0)
    for i in range(n2):
        for k in range(len(OSPLIT)):
            out_copy(i, k).wait()


@jax.jit
def pallas_gated_mix__linear_attn_block__mixer_s_mlp__prompt_kernel(
    A_x, A_wqkv, A_wo, B_x, B_w1, B_w2, B_w3, B_w4, gate_w,
):
    hbm = pl.BlockSpec(memory_space=pltpu.HBM)
    n2 = S // T2
    scratch = [
        pltpu.VMEM((S, D), BF),
        pltpu.VMEM((D, D), BF),
        pltpu.VMEM((D, D), BF),
        pltpu.VMEM((D, D), BF),
        pltpu.VMEM((D, D), BF),
        pltpu.VMEM((D, D), BF),
        pltpu.VMEM((D, D), BF),
        pltpu.VMEM((F, D), BF),
        pltpu.VMEM((F, D), BF),
        pltpu.VMEM((D,), BF),
        pltpu.VMEM((5, S + 2 * HALO, 128), F32),
        pltpu.VMEM((D, D), BF),
        pltpu.VMEM((6, D, 128), F32),
        pltpu.VMEM((D, 128), F32),
        pltpu.VMEM((D, D), BF),
        pltpu.VMEM((D, 128), F32),
        pltpu.VMEM((D, D), F32),
        pltpu.VMEM((D, 128), F32),
        pltpu.VMEM((S, D), F32),
        pltpu.VMEM((S, D), BF),
        pltpu.VMEM((S, D), BF),
        pltpu.SemaphoreType.DMA((len(XSEG),)),
        pltpu.SemaphoreType.DMA((10,)),
        pltpu.SemaphoreType.DMA((n2 * len(OSPLIT),)),
    ]
    return pl.pallas_call(
        _kernel,
        out_shape=jax.ShapeDtypeStruct((1, S, D), BF),
        in_specs=[hbm] * 8,
        out_specs=hbm,
        scratch_shapes=scratch,
        compiler_params=pltpu.CompilerParams(vmem_limit_bytes=100 * 1024 * 1024),
    )(A_x, A_wqkv, A_wo, B_w1, B_w2, B_w3.T, B_w4, gate_w)
```

```python
import jax
import jax.numpy as jnp
from jax import lax
import jax.experimental.pallas as pl
import jax.experimental.pallas.tpu as pltpu

S = 2048
D = 640
F = 1728
FM = 1664
H = 32
DH = 20
XSEG = [(0, 256), (256, 768), (768, 2048)]
X0 = XSEG[0][1]
W1A = 256
HC = 128
TB = 512
MCH = [128] * 15 + [64, 64]
T2 = 512
OSPLIT = [(0, 256), (256, 384), (384, 448), (448, 512)]
LNL = 64
HALO = 8
RB = 16
BF = jnp.bfloat16
F32 = jnp.float32

_C1 = 0.7978845608028654
_C2 = 0.7978845608028654 * 0.044715

_WIN = [(0, 144), (112, 272), (240, 400), (368, 528), (496, 640)]


def _gelu2(x):
    return x * (1.0 + jnp.tanh(x * (_C1 + _C2 * (x * x))))


def _gelu(x):
    return 0.5 * _gelu2(x)


def _phi(t):
    return jnp.where(t > 0, t + 1.0, jnp.exp(t)) + 1e-6


def _ln_stats(x):
    m = jnp.mean(x, axis=-1, keepdims=True)
    xc = x - m
    v = jnp.mean(xc * xc, axis=-1, keepdims=True)
    rstd = jnp.exp(-0.5 * jnp.log(v + 1e-5))
    return m, xc, rstd


def _ln(x):
    _, xc, rstd = _ln_stats(x)
    return xc * rstd


def _dot(a, b):
    return jnp.dot(a, b, preferred_element_type=F32)


def _dot_nt(a, b):
    return lax.dot_general(a, b, (((1,), (1,)), ((), ())), preferred_element_type=F32)


def _kernel(ax_hbm, wqkv_hbm, wo_hbm, w1_hbm, w2_hbm, w3_hbm, w4_hbm, gw_hbm,
            out_hbm,
            ax, wq, wk, wv, wo, w1, w2, w3, w4, gwv,
            hbuf, wqtp, tmp, tq, mp, zp, pacc, zacc, x1s, lns, outv,
            sem_ax, sem_w, sem_out):
    n2 = S // T2

    def ax_copy(i):
        lo, hi = XSEG[i]
        return pltpu.make_async_copy(ax_hbm.at[0, pl.ds(lo, hi - lo), :],
                                     ax.at[pl.ds(lo, hi - lo), :], sem_ax.at[i])

    def out_copy(i, k):
        lo, hi = OSPLIT[k]
        return pltpu.make_async_copy(outv.at[pl.ds(i * T2 + lo, hi - lo), :],
                                     out_hbm.at[0, pl.ds(i * T2 + lo, hi - lo), :],
                                     sem_out.at[i * len(OSPLIT) + k])

    wk_copy = pltpu.make_async_copy(wqkv_hbm.at[:, pl.ds(D, D)], wk, sem_w.at[0])
    w1a_copy = pltpu.make_async_copy(w1_hbm.at[:, pl.ds(0, W1A)], w1.at[:, pl.ds(0, W1A)], sem_w.at[1])
    w1b_copy = pltpu.make_async_copy(w1_hbm.at[:, pl.ds(W1A, D - W1A)], w1.at[:, pl.ds(W1A, D - W1A)],
                                     sem_w.at[9])
    wq_copy = pltpu.make_async_copy(wqkv_hbm.at[:, pl.ds(0, D)], wq, sem_w.at[2])
    wv_copy = pltpu.make_async_copy(wqkv_hbm.at[:, pl.ds(2 * D, D)], wv, sem_w.at[3])
    wo_copy = pltpu.make_async_copy(wo_hbm, wo, sem_w.at[4])
    w2_copy = pltpu.make_async_copy(w2_hbm, w2, sem_w.at[5])
    w3_copy = pltpu.make_async_copy(w3_hbm, w3, sem_w.at[6])
    w4_copy = pltpu.make_async_copy(w4_hbm, w4, sem_w.at[7])
    gw_copy = pltpu.make_async_copy(gw_hbm, gwv, sem_w.at[8])

    ax_copy(0).start()
    w1a_copy.start()
    w1b_copy.start()
    ax_copy(1).start()
    ax_copy(2).start()
    wk_copy.start()
    late = [w2_copy, wv_copy, wo_copy, gw_copy, w3_copy, w4_copy]

    for cc in range(5):
        hbuf[cc, pl.ds(0, HALO), :] = jnp.zeros((HALO, 128), F32)
        hbuf[cc, pl.ds(HALO + S, HALO), :] = jnp.zeros((HALO, 128), F32)
    pacc[...] = jnp.zeros((D, D), F32)
    zacc[...] = jnp.zeros((D, 128), F32)

    def h_chunk(r0, cs1):
        y = _dot(ax[r0:r0 + HC, :], w1[...])
        for rb in range(0, HC, RB):
            r = r0 + rb
            m, _, rstd = _ln_stats(ax[r:r + RB, :].astype(F32))
            h = _gelu((y[rb:rb + RB, :] - m * cs1) * rstd)
            for cc in range(5):
                hbuf[cc, HALO + r:HALO + r + RB, :] = h[:, 128 * cc:128 * (cc + 1)]

    def wq_t(cc):
        c0 = cc * 128 if isinstance(cc, int) else pl.multiple_of(cc * 128, 128)
        tq[...] = wq[pl.ds(c0, 128), :].astype(F32).T
        for d in range(DH):
            wqtp[d * H:(d + 1) * H, pl.ds(c0, 128)] = tq[pl.ds(d, H, stride=DH), :].astype(BF)

    ax_copy(0).wait()
    ln0 = jnp.concatenate(
        [_ln(ax[rb:rb + RB, :].astype(F32)).astype(BF) for rb in range(0, X0, RB)]
        + [jnp.ones((16, D), BF)], axis=0)
    w1a_copy.wait()
    y0a = _dot(ln0, w1[:, 0:W1A])
    for cc in range(W1A // 128):
        hbuf[cc, HALO:HALO + X0, :] = _gelu(y0a[0:X0, 128 * cc:128 * (cc + 1)])
    w1b_copy.wait()
    y0b = _dot(ln0, w1[:, W1A:D])
    for cc in range(W1A // 128, 5):
        hbuf[cc, HALO:HALO + X0, :] = _gelu(y0b[0:X0, 128 * cc - W1A:128 * (cc + 1) - W1A])
    cs1 = jnp.concatenate([y0a[X0:X0 + 1], y0b[X0:X0 + 1]], axis=1)
    ax_copy(1).wait()
    wq_copy.start()
    for r0 in range(XSEG[1][0], XSEG[1][1], HC):
        h_chunk(r0, cs1)
    ax_copy(2).wait()
    for r0 in range(XSEG[2][0], XSEG[2][1], HC):
        h_chunk(r0, cs1)
    wk_copy.wait()
    wq_copy.wait()

    def p1(i, carry):
        @pl.when(i == 1)
        def _():
            for cp in late:
                cp.start()
        r0 = pl.multiple_of(i * TB, TB)
        xa = ax[pl.ds(r0, TB), :]
        pkb = _phi(_dot(xa, wk[...])).T.astype(BF)
        pkf = pkb.astype(F32)
        zs = pkf[:, 0:128]
        for c in range(1, TB // 128):
            zs = zs + pkf[:, c * 128:(c + 1) * 128]
        zacc[...] += zs
        pacc[...] += _dot(pkb, xa)
        wq_t(i)
        return carry

    lax.fori_loop(0, S // TB, p1, 0)

    wv_copy.wait()
    wo_copy.wait()
    w2_copy.wait()

    def ln_rows(r0, n):
        for rb in range(0, n, RB):
            lns[r0 + rb:r0 + rb + RB, :] = _ln(x1s[r0 + rb:r0 + rb + RB, :]).astype(BF)

    offs = [sum(MCH[:k]) for k in range(len(MCH))]
    todo = list(range(len(MCH)))

    def x1_chunks(count):
        for _ in range(count):
            k = todo.pop(0)
            r0, n = offs[k], MCH[k]
            lane = lax.broadcasted_iota(jnp.int32, (n, 128), 1)

            def hw(off, cc):
                return hbuf[cc, pl.ds(r0 + HALO + off, n), :]
            t0 = hw(-1, 0)
            t1 = jnp.where(lane < 32, hw(-1, 1), hw(1, 1))
            t2 = jnp.where(lane < 64, hw(1, 2), hw(-2, 2))
            t3 = jnp.where(lane < 96, hw(-2, 3), hw(2, 3))
            t4 = hw(2, 4)
            hs = jnp.concatenate([t0, t1, t2, t3, t4], axis=1).astype(BF)
            x1s[r0:r0 + n, :] = ax[r0:r0 + n, :].astype(F32) + _dot(hs, w2[...])
            if r0 < S - LNL:
                ln_rows(r0, n)

    def kv_block(j):
        a, b = _WIN[j]
        g = _dot(pacc[a:b, :].astype(BF), wv[:, 128 * j:128 * (j + 1)])
        rh = ((lax.broadcasted_iota(jnp.int32, (b - a, 1), 0) + a) * 3277) >> 16
        ch = ((lax.broadcasted_iota(jnp.int32, (1, 128), 1) + 128 * j) * 3277) >> 16
        return jnp.where(rh == ch, g, 0.0).astype(BF)

    for c in range(5):
        tmp[c] = jnp.zeros((D, 128), F32)
    tmp[5] = zacc[...]
    x1_chunks(2)
    kv = [kv_block(j) for j in range(5)]
    x1_chunks(2)
    for j in range(5):
        a, b = _WIN[j]
        mj = _dot(kv[j], wo[128 * j:128 * (j + 1), :])
        for c in range(5):
            tmp[c, a:b, :] += mj[:, 128 * c:128 * (c + 1)]
    for d in range(DH):
        zp[d * H:(d + 1) * H, :] = tmp[5, pl.ds(d, H, stride=DH), :]
    zrow = jnp.sum(zp[...].T, axis=0, keepdims=True)
    x1_chunks(2)
    for c in range(5):
        for d in range(DH):
            mp[d * H:(d + 1) * H, 128 * c:128 * (c + 1)] = tmp[c, pl.ds(d, H, stride=DH), :].astype(BF)
    wq_t(4)
    x1_chunks(len(todo))

    w3_copy.wait()
    w4_copy.wait()
    gw_copy.wait()
    gw = gwv[...].astype(F32).reshape(1, D)

    def p2(i, carry):
        r0 = pl.multiple_of(i * T2, T2)
        xa = ax[pl.ds(r0, T2), :]
        pq = _phi(_dot_nt(xa, wqtp[...]))
        s = pq * zrow
        den = s[:, 0:128]
        for c in range(1, 5):
            den = den + s[:, c * 128:(c + 1) * 128]
        den = den + pltpu.roll(den, 32, 1)
        den = den + pltpu.roll(den, 64, 1)
        den = den + 1e-6
        g = jax.nn.sigmoid(jnp.sum(xa.astype(F32) * gw, axis=-1, keepdims=True))
        r = g / den
        pqn = jnp.concatenate([pq[:, c * 128:(c + 1) * 128] * r for c in range(5)], axis=1).astype(BF)
        ln = lns[pl.ds(r0, T2), :]
        hid = _gelu2(_dot_nt(ln, w3[0:FM, :])).astype(BF)
        hid_t = _gelu2(_dot_nt(w3[FM:F, :], ln)).T.astype(BF)
        for k, (lo, hi) in enumerate(OSPLIT):
            a = _dot(pqn[lo:hi], mp[...])
            h2 = _dot(hid[lo:hi], w4[0:FM, :]) + _dot(hid_t[lo:hi], w4[FM:F, :])
            rr = pl.multiple_of(r0 + lo, 64)
            b = x1s[pl.ds(rr, hi - lo), :] + 0.5 * h2
            outv[pl.ds(rr, hi - lo), :] = (a + (1.0 - g[lo:hi]) * b).astype(BF)
            out_copy(i, k).start()
        ln_rows(S - LNL, LNL)
        return carry

    lax.fori_loop(0, n2, p2, 0)
    for i in range(n2):
        for k in range(len(OSPLIT)):
            out_copy(i, k).wait()


@jax.jit
def pallas_gated_mix__linear_attn_block__mixer_s_mlp__prompt_kernel(
    A_x, A_wqkv, A_wo, B_x, B_w1, B_w2, B_w3, B_w4, gate_w,
):
    hbm = pl.BlockSpec(memory_space=pltpu.HBM)
    n2 = S // T2
    scratch = [
        pltpu.VMEM((S, D), BF),
        pltpu.VMEM((D, D), BF),
        pltpu.VMEM((D, D), BF),
        pltpu.VMEM((D, D), BF),
        pltpu.VMEM((D, D), BF),
        pltpu.VMEM((D, D), BF),
        pltpu.VMEM((D, D), BF),
        pltpu.VMEM((F, D), BF),
        pltpu.VMEM((F, D), BF),
        pltpu.VMEM((D,), BF),
        pltpu.VMEM((5, S + 2 * HALO, 128), F32),
        pltpu.VMEM((D, D), BF),
        pltpu.VMEM((6, D, 128), F32),
        pltpu.VMEM((D, 128), F32),
        pltpu.VMEM((D, D), BF),
        pltpu.VMEM((D, 128), F32),
        pltpu.VMEM((D, D), F32),
        pltpu.VMEM((D, 128), F32),
        pltpu.VMEM((S, D), F32),
        pltpu.VMEM((S, D), BF),
        pltpu.VMEM((S, D), BF),
        pltpu.SemaphoreType.DMA((len(XSEG),)),
        pltpu.SemaphoreType.DMA((10,)),
        pltpu.SemaphoreType.DMA((n2 * len(OSPLIT),)),
    ]
    return pl.pallas_call(
        _kernel,
        out_shape=jax.ShapeDtypeStruct((1, S, D), BF),
        in_specs=[hbm] * 8,
        out_specs=hbm,
        scratch_shapes=scratch,
        compiler_params=pltpu.CompilerParams(vmem_limit_bytes=100 * 1024 * 1024),
    )(A_x, A_wqkv, A_wo, B_w1, B_w2, B_w3.T, B_w4, gate_w)
```
